```python
import os as _os
_os.environ.setdefault("JAX_PLATFORMS", "cpu")
import jax
import jax.numpy as jnp

def _softmax(x, axis=-1):
    return jax.nn.softmax(x, axis=axis)
def _gelu(x):
    return jax.nn.gelu(x, approximate=True)
def _silu(x):
    return jax.nn.silu(x)
def _sigmoid(x):
    return jax.nn.sigmoid(x)
def _layernorm(x, axis=-1, eps=1e-5):
    m = jnp.mean(x, axis=axis, keepdims=True)
    v = jnp.var(x, axis=axis, keepdims=True)
    return (x - m) / jnp.sqrt(v + eps)
def _scatter_add(tgt, idx, src, axis=0):
    return tgt.at[idx].add(src)
def _segment_sum(src, seg, n):
    return jax.ops.segment_sum(src, seg, n)
class _Rng:
    def __init__(self, key):
        self._k = key
    def _next(self):
        self._k, sub = jax.random.split(self._k)
        return sub
    def normal(self, shape):
        return jax.random.normal(self._next(), shape, dtype=jnp.bfloat16)
    def randint(self, lo, hi, shape):
        return jax.random.randint(self._next(), shape, lo, hi, dtype=jnp.int32)
    def uniform(self, shape, lo=0.0, hi=1.0):
        return jax.random.uniform(self._next(), shape, jnp.bfloat16, lo, hi)
    def permutation(self, n):
        return jax.random.permutation(self._next(), n)


kernel_name = 'gated_mix__mha_block__mha_block__prompt'

def setup_inputs():
    _rng = _Rng(jax.random.key(int.from_bytes(__import__("os").urandom(4), "little")))
    _w = (lambda a: (lambda t: t.astype(jnp.bfloat16) if jnp.issubdtype(t.dtype, jnp.floating) else t)(jnp.asarray(a)))
    def _A_setup():
        B, S, D, H = 1, 2048, 448, 16
        return {
            "x": _w((lambda *s: _rng.normal(s) * 0.05)(B, S, D)),
            "wqkv": _w((lambda *s: _rng.normal(s) * 0.4)(D, 3 * D)),
            "wo": _w((lambda *s: _rng.normal(s) * 0.05)(D, D)),
        }
    _A_in = _A_setup()

    def _B_setup():
        B, S, D, H = 1, 2048, 448, 16
        return {
            "x": _w((lambda *s: _rng.normal(s) * 0.05)(B, S, D)),
            "wqkv": _w((lambda *s: _rng.normal(s) * 0.4)(D, 3 * D)),
            "wo": _w((lambda *s: _rng.normal(s) * 0.05)(D, D)),
        }
    _B_in = _B_setup()

    return {
        "A_x": _A_in["x"],
        "A_wqkv": _A_in["wqkv"],
        "A_wo": _A_in["wo"],
        "B_x": _B_in["x"],
        "B_wqkv": _B_in["wqkv"],
        "B_wo": _B_in["wo"],
        "gate_w": _w((lambda *s: _rng.normal(s) * 0.05)(448) * 16.0),
    }

def reference(A_x, A_wqkv, A_wo, B_x, B_wqkv, B_wo, gate_w):
    def _A_ref(x, wqkv, wo):
        B, S, D = x.shape
        H = 16
        Dh = D // H
        qkv = (lambda x, *d: x.transpose(*d))((x @ wqkv).reshape(B, S, 3, H, Dh), 2, 0, 3, 1, 4)
        q, k, v = qkv[0], qkv[1], qkv[2]
        scores = jnp.einsum("bhqd,bhkd->bhqk", q, k) * (Dh ** -0.5)
        p = _softmax(scores, axis=-1)
        o = jnp.einsum("bhqk,bhkd->bhqd", p, v)
        return (lambda x, *d: x.transpose(*d))(o, 0, 2, 1, 3).reshape(B, S, D) @ wo

    def _B_ref(x, wqkv, wo):
        B, S, D = x.shape
        H = 16
        Dh = D // H
        qkv = (lambda x, *d: x.transpose(*d))((x @ wqkv).reshape(B, S, 3, H, Dh), 2, 0, 3, 1, 4)
        q, k, v = qkv[0], qkv[1], qkv[2]
        scores = jnp.einsum("bhqd,bhkd->bhqk", q, k) * (Dh ** -0.5)
        p = _softmax(scores, axis=-1)
        o = jnp.einsum("bhqk,bhkd->bhqd", p, v)
        return (lambda x, *d: x.transpose(*d))(o, 0, 2, 1, 3).reshape(B, S, D) @ wo

    x = A_x
    g = _sigmoid((x * gate_w).sum(-1, keepdims=True))
    a = _A_ref(x, A_wqkv, A_wo)
    b = _B_ref(x, B_wqkv, B_wo)
    return g * a + (1 - g) * b
```

```python
import functools, math
import jax, jax.numpy as jnp
from jax import lax
from jax.experimental import pallas as pl
from jax.experimental.pallas import tpu as pltpu

S = 2048; D = 448; H = 16; DH = 28; HP = 32; NH = 2 * H
TQ = 512
NQ = S // TQ
NSTEP = NH * NQ
CK = 256
NC = S // CK
NP = NH * HP

def _kernel(x_ref, wa_ref, wb_ref, woa_ref, wob_ref, gw_ref, o_ref,
            wT_scr, wo_scr, k_scr, qT_scr, vT_scr, oT_scr, g_scr, sa, sb, ma, mb):
    f32 = jnp.float32
    bf16 = jnp.bfloat16
    wT_scr[...] = jnp.zeros_like(wT_scr)
    wo_scr[...] = jnp.zeros_like(wo_scr)
    for br, (w_ref, wo_ref) in enumerate(((wa_ref, woa_ref), (wb_ref, wob_ref))):
        wt = w_ref[...].astype(f32).T
        for part, base in ((0, 0), (2, NP), (1, 2 * NP)):
            for h in range(H):
                src = part * D + h * DH
                dst = base + (br * H + h) * HP
                wT_scr[dst:dst + DH, :] = wt[src:src + DH, :].astype(bf16)
        wo = wo_ref[...].astype(f32)
        for h in range(H):
            dst = (br * H + h) * HP
            wo_scr[dst:dst + DH, :] = wo[h * DH:(h + 1) * DH, :]

    xT = x_ref[...]
    nt = (((1,), (1,)), ((), ()))
    qscale = (DH ** -0.5) * math.log2(math.e)
    qT = jnp.dot(wT_scr[0:NP, :], xT, preferred_element_type=f32)
    qT_scr[...] = (qT * qscale).astype(bf16)
    x = xT.T
    k_scr[...] = lax.dot_general(x, wT_scr[2 * NP:3 * NP, :], nt, preferred_element_type=f32).astype(bf16)
    vT = jnp.dot(wT_scr[NP:2 * NP, :], xT, preferred_element_type=f32)
    row = lax.broadcasted_iota(jnp.int32, vT.shape, 0)
    vT_scr[...] = jnp.where((row % HP) == DH, 1.0, vT).astype(bf16)
    gw = jnp.broadcast_to(gw_ref[...], (16, D))
    gl = jnp.dot(gw, xT, preferred_element_type=f32)
    g = jax.nn.sigmoid(gl[0:8, :])
    g_scr[0:8, :] = g
    g_scr[8:16, :] = 1.0 - g

    def get_qm(i):
        h = i // NQ
        t = i % NQ
        grp = h // 4
        j = h % 4
        q0 = pl.multiple_of(t * TQ, TQ)
        qg = qT_scr[pl.ds(pl.multiple_of(grp * 128, 128), 128), pl.ds(q0, TQ)]
        r = lax.broadcasted_iota(jnp.int32, qg.shape, 0)
        return jnp.where((r // HP) == j, qg, jnp.zeros_like(qg)), pl.multiple_of(grp * 128, 128)

    def step(i_next, s_next, m_next, i_cur, s_cur, m_cur):
        qm, koff = get_qm(i_next)
        if i_cur is not None:
            h = i_cur // NQ
            t = i_cur % NQ
            q0 = pl.multiple_of(t * TQ, TQ)
            hoff = pl.multiple_of(h * HP, HP)
            mc = m_cur[...]
            o = jnp.zeros((HP, TQ), f32)
        m = None
        for c in range(NC):
            kc = k_scr[c * CK:(c + 1) * CK, pl.ds(koff, 128)]
            s = jnp.dot(kc, qm, preferred_element_type=f32)
            s_next[c * CK:(c + 1) * CK, :] = s
            mm = jnp.max(s.reshape(CK // 8, 8, TQ), axis=0)
            m = mm if m is None else jnp.maximum(m, mm)
            if i_cur is not None:
                p = jnp.exp2(s_cur[c * CK:(c + 1) * CK, :] - mc).astype(bf16)
                vh = vT_scr[pl.ds(hoff, HP), c * CK:(c + 1) * CK]
                o = o + jnp.dot(vh, p, preferred_element_type=f32)
        m_next[...] = jnp.max(m, axis=0, keepdims=True)
        if i_cur is not None:
            l = o[DH:DH + 1, :]
            br = h // H
            gg = g_scr[pl.ds(pl.multiple_of(br * 8, 8), 1), pl.ds(q0, TQ)]
            oT_scr[pl.ds(hoff, HP), pl.ds(q0, TQ)] = (o * (gg / l)).astype(bf16)

    step(0, sa, ma, None, None, None)
    def body(k, c):
        i = 2 * k
        step(i + 1, sb, mb, i, sa, ma)
        step(jnp.minimum(i + 2, NSTEP - 1), sa, ma, i + 1, sb, mb)
        return c
    lax.fori_loop(0, NSTEP // 2, body, 0)

    woT = wo_scr[...].T.astype(bf16)
    for t in range(S // 512):
        outT = jnp.dot(woT, oT_scr[:, t * 512:(t + 1) * 512], preferred_element_type=f32)
        o_ref[:, t * 512:(t + 1) * 512] = outT.astype(o_ref.dtype)


@jax.jit
def pallas_gated_mix__mha_block__mha_block__prompt_kernel(A_x, A_wqkv, A_wo, B_x, B_wqkv, B_wo, gate_w):
    x = A_x.reshape(S, D).T
    out = pl.pallas_call(
        _kernel,
        out_shape=jax.ShapeDtypeStruct((D, S), jnp.bfloat16),
        scratch_shapes=[
            pltpu.VMEM((3 * NP, D), jnp.bfloat16),
            pltpu.VMEM((NP, D), jnp.float32),
            pltpu.VMEM((S, NP), jnp.bfloat16),
            pltpu.VMEM((NP, S), jnp.bfloat16),
            pltpu.VMEM((NP, S), jnp.bfloat16),
            pltpu.VMEM((NP, S), jnp.bfloat16),
            pltpu.VMEM((16, S), jnp.float32),
            pltpu.VMEM((S, TQ), jnp.float32),
            pltpu.VMEM((S, TQ), jnp.float32),
            pltpu.VMEM((1, TQ), jnp.float32),
            pltpu.VMEM((1, TQ), jnp.float32),
        ],
        compiler_params=pltpu.CompilerParams(vmem_limit_bytes=100 * 1024 * 1024),
    )(x, A_wqkv, B_wqkv, A_wo, B_wo, gate_w.reshape(1, D))
    return out.T.reshape(1, S, D)
```

```python
import functools, math
import jax, jax.numpy as jnp
from jax import lax
from jax.experimental import pallas as pl
from jax.experimental.pallas import tpu as pltpu

S = 2048; D = 448; H = 16; DH = 28; HP = 32; NH = 2 * H
TQ = 1024
NQ = S // TQ
NSTEP = NH * NQ
CK = 128
NC = S // CK
NP = NH * HP
BP = H * HP
UNROLL = 4
LAG = 1
ORDER = 0
OT = 512
GW = 4 * DH
XC = 512
NXC = S // XC
WQ = 512
GROW = DH + 1

def _kernel(x_hbm, wa_hbm, wb_hbm, woa_hbm, wob_hbm, gw_hbm, o_hbm,
            x_v, wa_v, wb_v, woa_v, wob_v, gw_v, o_v, sem_in, sem_out,
            wv_scr, wo_scr, woT_scr, k_scr, qT_scr, vT_scr, oT_scr, g_scr, sa):
    f32 = jnp.float32
    bf16 = jnp.bfloat16
    xcs = [(0, 512), (512, 1024), (1024, 1536), (1536, 2048)]
    pairs = [(wa_hbm.at[:, 0:WQ], wa_v.at[:, 0:WQ])]
    pairs += [(x_hbm.at[:, lo:hi], x_v.at[:, lo:hi]) for lo, hi in xcs]
    pairs += [(wa_hbm.at[:, WQ:3 * D], wa_v.at[:, WQ:3 * D]), (gw_hbm, gw_v), (wb_hbm, wb_v),
              (woa_hbm, woa_v), (wob_hbm, wob_v)]
    copies = [pltpu.make_async_copy(s_, d_, sem_in.at[n]) for n, (s_, d_) in enumerate(pairs)]
    for cp in copies:
        cp.start()
    c_waq = copies[0]; c_x = copies[1:1 + len(xcs)]
    c_war, c_gw, c_wb, c_woa, c_wob = copies[1 + len(xcs):]
    wv_scr[...] = jnp.zeros_like(wv_scr)
    wo_scr[...] = jnp.zeros_like(wo_scr)
    k_scr[...] = jnp.zeros_like(k_scr)

    nt = (((1,), (1,)), ((), ()))
    qscale = (DH ** -0.5) * math.log2(math.e)

    c_waq.wait()
    wqT = wa_v[:, 0:WQ].astype(f32).T[0:D, :].astype(bf16)
    for n, (lo, hi) in enumerate(xcs):
        c_x[n].wait()
        if n == len(xcs) - 1 and True:
            c_war.wait()
            c_gw.wait()
        qT = jnp.dot(wqT, x_v[:, lo:hi], preferred_element_type=f32)
        qT_scr[0:D, lo:hi] = (qT * qscale).astype(bf16)
    if not True:
        c_war.wait()
        c_gw.wait()
    xT = x_v[...]
    x = xT.T
    for br, w_v in enumerate((wa_v, wb_v)):
        wt32 = w_v[...].astype(f32).T
        wt = wt32[0:2 * D, :].astype(bf16)
        for h in range(H):
            src = 2 * D + h * DH
            wv_scr[h * HP:h * HP + DH, :] = wt32[src:src + DH, :].astype(bf16)
        if br == 0:
            wv_scr[GROW:GROW + 1, :] = gw_v[...]
        else:
            qT = jnp.dot(wt[0:D, :], xT, preferred_element_type=f32)
            qT_scr[br * D:(br + 1) * D, :] = (qT * qscale).astype(bf16)
        for g4 in range(4):
            kg = lax.dot_general(x, wt[D + g4 * GW:D + (g4 + 1) * GW, :], nt, preferred_element_type=f32)
            k_scr[:, (br * 4 + g4) * 128:(br * 4 + g4) * 128 + GW] = kg.astype(bf16)
        if br == 0:
            c_wb.wait()
            c_woa.wait()
            c_wob.wait()
        vT = jnp.dot(wv_scr[...], xT, preferred_element_type=f32)
        if br == 0:
            g = jax.nn.sigmoid(vT[GROW:GROW + 1, :])
            g_scr[0:1, :] = g
            g_scr[8:9, :] = 1.0 - g
        row = lax.broadcasted_iota(jnp.int32, vT.shape, 0) % HP
        vT = jnp.where(row == DH, 1.0, jnp.where(row > DH, 0.0, vT))
        vT_scr[br * BP:(br + 1) * BP, :] = vT.astype(bf16)
        if br == 0:
            for b2, wo_v in enumerate((woa_v, wob_v)):
                wo = wo_v[...].astype(f32)
                for h in range(H):
                    dst = (b2 * H + h) * HP
                    wo_scr[dst:dst + DH, :] = wo[h * DH:(h + 1) * DH, :]
            woT_scr[...] = wo_scr[...].T.astype(bf16)

    def get_qm(i):
        h = i // NQ
        t = i % NQ
        grp = h // 4
        j = h % 4
        q0 = pl.multiple_of(t * TQ, TQ)
        qg = qT_scr[pl.ds(pl.multiple_of(grp * GW, 16), GW), pl.ds(q0, TQ)]
        r = lax.broadcasted_iota(jnp.int32, qg.shape, 0)
        qm = jnp.where((r >= j * DH) & (r < (j + 1) * DH), qg, jnp.zeros_like(qg))
        qm = jnp.concatenate([qm, jnp.zeros((128 - GW, TQ), bf16)], axis=0)
        return qm, pl.multiple_of(grp * 128, 128)

    B = UNROLL * NC

    def run(i0, qk_items, sm_items, order):
        st = {}
        sbuf = {}
        def qk(u, c, to_scr):
            if ("q", u) not in st:
                st[("q", u)] = get_qm(jnp.minimum(i0 + u, NSTEP - 1))
            qm, koff = st[("q", u)]
            kc = k_scr[c * CK:(c + 1) * CK, pl.ds(koff, 128)]
            s = jnp.dot(kc, qm, preferred_element_type=f32)
            if to_scr:
                sa[c * CK:(c + 1) * CK, :] = s
            else:
                sbuf[(u, c)] = s
        def sm_pv(u, c, from_scr):
            i = i0 + u
            h = i // NQ
            hoff = pl.multiple_of(h * HP, HP)
            s = sa[c * CK:(c + 1) * CK, :] if from_scr else sbuf.pop((u, c))
            m, o = st.get(("s", u), (None, None))
            mm = jnp.max(s, axis=0, keepdims=True)
            m_new = mm if m is None else jnp.maximum(m, mm)
            p = jnp.exp2(s - m_new).astype(bf16)
            vh = vT_scr[pl.ds(hoff, HP), c * CK:(c + 1) * CK]
            pv = jnp.dot(vh, p, preferred_element_type=f32)
            o = pv if o is None else o * jnp.exp2(m - m_new) + pv
            st[("s", u)] = (m_new, o)
            if c == NC - 1:
                t = i % NQ
                q0 = pl.multiple_of(t * TQ, TQ)
                l = o[DH:DH + 1, :]
                br = h // H
                gg = g_scr[pl.ds(pl.multiple_of(br * 8, 8), 1), pl.ds(q0, TQ)]
                oT_scr[pl.ds(hoff, HP), pl.ds(q0, TQ)] = (o * (gg / l)).astype(bf16)
        for n in range(max(len(qk_items), len(sm_items))):
            if order == 0 and n < len(qk_items):
                qk(*qk_items[n])
            if n < len(sm_items):
                sm_pv(*sm_items[n])
            if order == 1 and n < len(qk_items):
                qk(*qk_items[n])

    run(0, [(0, c, True) for c in range(LAG)], [], 0)
    def body(k, carry):
        i0 = UNROLL * k
        qk_items = [((n + LAG) // NC, (n + LAG) % NC, n + LAG >= B) for n in range(B)]
        sm_items = [(n // NC, n % NC, n < LAG) for n in range(B)]
        run(i0, qk_items, sm_items, ORDER)
        return carry
    lax.fori_loop(0, NSTEP // UNROLL, body, 0)

    woT = woT_scr[...]
    outs = []
    for t in range(S // OT):
        outT = jnp.dot(woT, oT_scr[:, t * OT:(t + 1) * OT], preferred_element_type=f32)
        o_v[:, t * OT:(t + 1) * OT] = outT.astype(o_v.dtype)
        cp = pltpu.make_async_copy(o_v.at[:, t * OT:(t + 1) * OT], o_hbm.at[:, t * OT:(t + 1) * OT], sem_out.at[t])
        cp.start()
        outs.append(cp)
    for cp in outs:
        cp.wait()


@jax.jit
def pallas_gated_mix__mha_block__mha_block__prompt_kernel(A_x, A_wqkv, A_wo, B_x, B_wqkv, B_wo, gate_w):
    x = A_x.reshape(S, D).T
    bf16 = jnp.bfloat16
    out = pl.pallas_call(
        _kernel,
        out_shape=jax.ShapeDtypeStruct((D, S), bf16),
        in_specs=[pl.BlockSpec(memory_space=pl.ANY)] * 6,
        out_specs=pl.BlockSpec(memory_space=pl.ANY),
        scratch_shapes=[
            pltpu.VMEM((D, S), bf16),
            pltpu.VMEM((D, 3 * D), bf16),
            pltpu.VMEM((D, 3 * D), bf16),
            pltpu.VMEM((D, D), bf16),
            pltpu.VMEM((D, D), bf16),
            pltpu.VMEM((1, D), bf16),
            pltpu.VMEM((D, S), bf16),
            pltpu.SemaphoreType.DMA((12,)),
            pltpu.SemaphoreType.DMA((S // OT,)),
            pltpu.VMEM((BP, D), bf16),
            pltpu.VMEM((NP, D), jnp.float32),
            pltpu.VMEM((D, NP), bf16),
            pltpu.VMEM((S, NP), bf16),
            pltpu.VMEM((2 * D, S), bf16),
            pltpu.VMEM((NP, S), bf16),
            pltpu.VMEM((NP, S), bf16),
            pltpu.VMEM((16, S), jnp.float32),
            pltpu.VMEM((LAG * CK, TQ), jnp.float32),
        ],
        compiler_params=pltpu.CompilerParams(vmem_limit_bytes=100 * 1024 * 1024),
    )(x, A_wqkv, B_wqkv, A_wo, B_wo, gate_w.reshape(1, D))
    return out.T.reshape(1, S, D)
```

```python
import functools, math
import jax, jax.numpy as jnp
from jax import lax
from jax.experimental import pallas as pl
from jax.experimental.pallas import tpu as pltpu

S = 2048; D = 448; H = 16; DH = 28; HP = 32; NH = 2 * H
TQ = 1024
NQ = S // TQ
NSTEP = NH * NQ
CK = 128
NC = S // CK
NP = NH * HP
BP = H * HP
UNROLL = 4
LAG = 1
OT = 512
GW = 4 * DH
WQ = 512

def _kernel(x_hbm, wa_hbm, wb_hbm, woa_hbm, wob_hbm, gw_hbm, o_hbm,
            x_v, wa_v, wb_v, woa_v, wob_v, gw_v, o_v, sem_in, sem_out,
            woT_scr, k_scr, qT_scr, vT_scr, oT_scr, g_scr, sa):
    f32 = jnp.float32
    bf16 = jnp.bfloat16
    xcs = [(0, 512), (512, 1024), (1024, 1536), (1536, 2048)]
    pairs = [(wa_hbm.at[:, 0:WQ], wa_v.at[:, 0:WQ])]
    pairs += [(x_hbm.at[:, lo:hi], x_v.at[:, lo:hi]) for lo, hi in xcs]
    pairs += [(wa_hbm.at[:, WQ:3 * D], wa_v.at[:, WQ:3 * D]), (gw_hbm, gw_v), (wb_hbm, wb_v),
              (woa_hbm, woa_v), (wob_hbm, wob_v)]
    copies = [pltpu.make_async_copy(s_, d_, sem_in.at[n]) for n, (s_, d_) in enumerate(pairs)]
    for cp in copies:
        cp.start()
    c_waq = copies[0]; c_x = copies[1:1 + len(xcs)]
    c_war, c_gw, c_wb, c_woa, c_wob = copies[1 + len(xcs):]

    nt = (((1,), (1,)), ((), ()))
    qscale = (DH ** -0.5) * math.log2(math.e)

    def store_q(br, qT, lo, hi):
        q16 = (qT * qscale).astype(bf16)
        r = lax.broadcasted_iota(jnp.int32, (GW, hi - lo), 0)
        zpad = jnp.zeros((128 - GW, hi - lo), bf16)
        for g4 in range(4):
            qg = q16[g4 * GW:(g4 + 1) * GW, :]
            for j in range(4):
                qm = jnp.where((r >= j * DH) & (r < (j + 1) * DH), qg, jnp.zeros_like(qg))
                qT_scr[br * H + g4 * 4 + j, :, lo:hi] = jnp.concatenate([qm, zpad], axis=0)

    c_waq.wait()
    wqT = wa_v[:, 0:WQ].astype(f32).T[0:D, :].astype(bf16)
    for n, (lo, hi) in enumerate(xcs):
        c_x[n].wait()
        if n == len(xcs) - 1:
            c_war.wait()
            c_gw.wait()
        qT = jnp.dot(wqT, x_v[:, lo:hi], preferred_element_type=f32)
        store_q(0, qT, lo, hi)
    xT = x_v[...]
    x = xT.T
    for br, w_v in enumerate((wa_v, wb_v)):
        wt = w_v[...].astype(f32).T.astype(bf16)
        if br == 1:
            qT = jnp.dot(wt[0:D, :], xT, preferred_element_type=f32)
            store_q(1, qT, 0, S)
        for g4 in range(4):
            kg = lax.dot_general(x, wt[D + g4 * GW:D + g4 * GW + 128, :], nt, preferred_element_type=f32)
            k_scr[:, (br * 4 + g4) * 128:(br * 4 + g4 + 1) * 128] = kg.astype(bf16)
        wvT = wt[2 * D:3 * D, :]
        if br == 0:
            c_wb.wait()
            c_woa.wait()
            c_wob.wait()
            wvT = jnp.concatenate([wvT, jnp.broadcast_to(gw_v[...], (16, D))], axis=0)
        vT = jnp.dot(wvT, xT, preferred_element_type=f32)
        if br == 0:
            g = jax.nn.sigmoid(vT[D:D + 1, :])
            g_scr[0:1, :] = g
            g_scr[8:9, :] = 1.0 - g
        pad = jnp.where(lax.broadcasted_iota(jnp.int32, (HP - DH, S), 0) == 0, 1.0, 0.0)
        for h in range(H):
            dst = (br * H + h) * HP
            vT_scr[dst:dst + HP, :] = jnp.concatenate([vT[h * DH:(h + 1) * DH, :], pad], axis=0).astype(bf16)
        if br == 0:
            woT_scr[:, 0:D] = woa_v[...].astype(f32).T.astype(bf16)
            woT_scr[:, D:2 * D] = wob_v[...].astype(f32).T.astype(bf16)

    def step_ht(i):
        kk = i // UNROLL
        u = i % UNROLL
        return 2 * kk + u % 2, u // 2

    def get_qm(i):
        h, t = step_ht(i)
        q0 = pl.multiple_of(t * TQ, TQ)
        return qT_scr[h, :, pl.ds(q0, TQ)], pl.multiple_of((h // 4) * 128, 128)

    B = UNROLL * NC

    def run(k, qk_items, sm_items):
        i0 = UNROLL * k
        st = {}
        sbuf = {}
        def qk(u, c, to_scr):
            if ("q", u) not in st:
                st[("q", u)] = get_qm(jnp.minimum(i0 + u, NSTEP - 1))
            qm, koff = st[("q", u)]
            kc = k_scr[c * CK:(c + 1) * CK, pl.ds(koff, 128)]
            s = jnp.dot(kc, qm, preferred_element_type=f32)
            if to_scr:
                sa[c * CK:(c + 1) * CK, :] = s
            else:
                sbuf[(u, c)] = s
        def sm_pv(u, c, from_scr):
            h = 2 * k + u % 2
            hoff = pl.multiple_of(h * HP, HP)
            s = sa[c * CK:(c + 1) * CK, :] if from_scr else sbuf.pop((u, c))
            m, o = st.get(("s", u), (None, None))
            mm = jnp.max(s, axis=0, keepdims=True)
            m_new = mm if m is None else jnp.maximum(m, mm)
            p = jnp.exp2(s - m_new).astype(bf16)
            vh = vT_scr[pl.ds(hoff, HP), c * CK:(c + 1) * CK]
            pv = jnp.dot(vh, p, preferred_element_type=f32)
            o = pv if o is None else o * jnp.exp2(m - m_new) + pv
            st[("s", u)] = (m_new, o)
            if c == NC - 1:
                q0 = (u // 2) * TQ
                l = o[DH:DH + 1, :]
                br = (2 * k) // H
                gg = g_scr[pl.ds(pl.multiple_of(br * 8, 8), 1), q0:q0 + TQ]
                on = o[0:DH, :] * (gg / l)
                if u % 2 == 0:
                    st["even"] = on
                else:
                    both = jnp.concatenate([st.pop("even"), on], axis=0)
                    oT_scr[pl.ds(pl.multiple_of(k * 2 * DH, 8), 2 * DH), q0:q0 + TQ] = both
        for n in range(max(len(qk_items), len(sm_items))):
            if n < len(qk_items):
                qk(*qk_items[n])
            if n < len(sm_items):
                sm_pv(*sm_items[n])

    run(0, [(0, c, True) for c in range(LAG)], [])
    def body(k, carry):
        qk_items = [((n + LAG) // NC, (n + LAG) % NC, n + LAG >= B) for n in range(B)]
        sm_items = [(n // NC, n % NC, n < LAG) for n in range(B)]
        run(k, qk_items, sm_items)
        return carry
    lax.fori_loop(0, NSTEP // UNROLL, body, 0)

    woT = woT_scr[...]
    outs = []
    for t in range(S // OT):
        outT = jnp.dot(woT, oT_scr[:, t * OT:(t + 1) * OT].astype(bf16), preferred_element_type=f32)
        o_v[:, t * OT:(t + 1) * OT] = outT.astype(o_v.dtype)
        cp = pltpu.make_async_copy(o_v.at[:, t * OT:(t + 1) * OT], o_hbm.at[:, t * OT:(t + 1) * OT], sem_out.at[t])
        cp.start()
        outs.append(cp)
    for cp in outs:
        cp.wait()


@jax.jit
def pallas_gated_mix__mha_block__mha_block__prompt_kernel(A_x, A_wqkv, A_wo, B_x, B_wqkv, B_wo, gate_w):
    x = A_x.reshape(S, D).T
    bf16 = jnp.bfloat16
    out = pl.pallas_call(
        _kernel,
        out_shape=jax.ShapeDtypeStruct((D, S), bf16),
        in_specs=[pl.BlockSpec(memory_space=pl.ANY)] * 6,
        out_specs=pl.BlockSpec(memory_space=pl.ANY),
        scratch_shapes=[
            pltpu.VMEM((D, S), bf16),
            pltpu.VMEM((D, 3 * D), bf16),
            pltpu.VMEM((D, 3 * D), bf16),
            pltpu.VMEM((D, D), bf16),
            pltpu.VMEM((D, D), bf16),
            pltpu.VMEM((1, D), bf16),
            pltpu.VMEM((D, S), bf16),
            pltpu.SemaphoreType.DMA((10,)),
            pltpu.SemaphoreType.DMA((S // OT,)),
            pltpu.VMEM((D, 2 * D), bf16),
            pltpu.VMEM((S, NP), bf16),
            pltpu.VMEM((NH, 128, S), bf16),
            pltpu.VMEM((NP, S), bf16),
            pltpu.VMEM((2 * D, S), jnp.float32),
            pltpu.VMEM((16, S), jnp.float32),
            pltpu.VMEM((LAG * CK, TQ), jnp.float32),
        ],
        compiler_params=pltpu.CompilerParams(vmem_limit_bytes=100 * 1024 * 1024),
    )(x, A_wqkv, B_wqkv, A_wo, B_wo, gate_w.reshape(1, D))
    return out.T.reshape(1, S, D)
```

```python
import math

import jax
import jax.numpy as jnp
from jax import lax
from jax.experimental import pallas as pl
from jax.experimental.pallas import tpu as pltpu

S = 2048
D = 448
H = 16
DH = 28
HP = 32
NH = 2 * H
GW = 4 * DH
TQ = 1024
NSTEP = NH * (S // TQ)
CK = 128
NC = S // CK
UNROLL = 4
NB = UNROLL * NC
WQ = 512
XCS = ((0, 512), (512, 1024), (1024, 1536), (1536, 2048))
OTS = ((0, 512), (512, 1024), (1024, 1536), (1536, 1920), (1920, 2048))


def _kernel(x_hbm, wa_hbm, wb_hbm, woa_hbm, wob_hbm, gw_hbm, o_hbm,
            x_v, wa_v, wb_v, woa_v, wob_v, gw_v, o_v, sem_in, sem_out,
            woT_scr, k_scr, q_scr, vT_scr, oT_scr, g_scr, s_carry):
    f32 = jnp.float32
    bf16 = jnp.bfloat16

    pairs = [(wa_hbm.at[:, 0:WQ], wa_v.at[:, 0:WQ])]
    pairs += [(x_hbm.at[:, lo:hi], x_v.at[:, lo:hi]) for lo, hi in XCS]
    pairs += [(wa_hbm.at[:, WQ:3 * D], wa_v.at[:, WQ:3 * D]), (gw_hbm, gw_v), (wb_hbm, wb_v),
              (woa_hbm, woa_v), (wob_hbm, wob_v)]
    copies = [pltpu.make_async_copy(src, dst, sem_in.at[n]) for n, (src, dst) in enumerate(pairs)]
    for cp in copies:
        cp.start()
    c_waq = copies[0]
    c_x = copies[1:1 + len(XCS)]
    c_war, c_gw, c_wb, c_woa, c_wob = copies[1 + len(XCS):]

    qscale = (DH ** -0.5) * math.log2(math.e)

    def store_q(br, qT, lo, hi):
        q16 = (qT * qscale).astype(bf16)
        r = lax.broadcasted_iota(jnp.int32, (GW, hi - lo), 0)
        zpad = jnp.zeros((128 - GW, hi - lo), bf16)
        for g4 in range(4):
            qg = q16[g4 * GW:(g4 + 1) * GW, :]
            for j in range(4):
                qm = jnp.where((r >= j * DH) & (r < (j + 1) * DH), qg, jnp.zeros_like(qg))
                q_scr[br * H + g4 * 4 + j, :, lo:hi] = jnp.concatenate([qm, zpad], axis=0)

    c_waq.wait()
    wqT = wa_v[:, 0:WQ].astype(f32).T[0:D, :].astype(bf16)
    for n, (lo, hi) in enumerate(XCS):
        c_x[n].wait()
        if n == len(XCS) - 1:
            c_war.wait()
            c_gw.wait()
        store_q(0, jnp.dot(wqT, x_v[:, lo:hi], preferred_element_type=f32), lo, hi)
    xT = x_v[...]
    for br, w_v in enumerate((wa_v, wb_v)):
        wt = w_v[...].astype(f32).T.astype(bf16)
        kT = jnp.dot(wt[D:2 * D, :], xT, preferred_element_type=f32)
        kT = jnp.concatenate([kT, jnp.zeros((128 - GW, S), f32)], axis=0)
        for g4 in range(4):
            k_scr[:, (br * 4 + g4) * 128:(br * 4 + g4 + 1) * 128] = (
                kT[g4 * GW:g4 * GW + 128, :].T.astype(bf16))
        if br == 1:
            store_q(1, jnp.dot(wt[0:D, :], xT, preferred_element_type=f32), 0, S)
        wvT = wt[2 * D:3 * D, :]
        if br == 0:
            c_wb.wait()
            c_woa.wait()
            c_wob.wait()
            wvT = jnp.concatenate(
                [wvT, jnp.broadcast_to(gw_v[...].reshape(1, D), (16, D))], axis=0)
        vT = jnp.dot(wvT, xT, preferred_element_type=f32)
        if br == 0:
            g = jax.nn.sigmoid(vT[D:D + 1, :])
            g_scr[0:1, :] = g
            g_scr[8:9, :] = 1.0 - g
        pad = jnp.where(lax.broadcasted_iota(jnp.int32, (HP - DH, S), 0) == 0, 1.0, 0.0)
        for h in range(H):
            dst = (br * H + h) * HP
            vT_scr[dst:dst + HP, :] = jnp.concatenate(
                [vT[h * DH:(h + 1) * DH, :], pad], axis=0).astype(bf16)
        if br == 0:
            woT_scr[:, 0:D] = woa_v[...].astype(f32).T.astype(bf16)
            woT_scr[:, D:2 * D] = wob_v[...].astype(f32).T.astype(bf16)

    def get_q(i):
        u = i % UNROLL
        h = 2 * (i // UNROLL) + u % 2
        q0 = pl.multiple_of((u // 2) * TQ, TQ)
        return q_scr[h, :, pl.ds(q0, TQ)], pl.multiple_of((h // 4) * 128, 128)

    def run(k, qk_items, sm_items):
        st = {}
        sbuf = {}

        def qk(u, c, to_carry):
            if ("q", u) not in st:
                st[("q", u)] = get_q(jnp.minimum(UNROLL * k + u, NSTEP - 1))
            qm, koff = st[("q", u)]
            kc = k_scr[c * CK:(c + 1) * CK, pl.ds(koff, 128)]
            s = jnp.dot(kc, qm, preferred_element_type=f32)
            if to_carry:
                s_carry[...] = s
            else:
                sbuf[(u, c)] = s

        def sm_pv(u, c, from_carry):
            h = 2 * k + u % 2
            s = s_carry[...] if from_carry else sbuf.pop((u, c))
            m, o = st.get(("s", u), (None, None))
            mm = jnp.max(s, axis=0, keepdims=True)
            m_new = mm if m is None else jnp.maximum(m, mm)
            p = jnp.exp2(s - m_new).astype(bf16)
            vh = vT_scr[pl.ds(pl.multiple_of(h * HP, HP), HP), c * CK:(c + 1) * CK]
            pv = jnp.dot(vh, p, preferred_element_type=f32)
            o = pv if o is None else o * jnp.exp2(m - m_new) + pv
            st[("s", u)] = (m_new, o)
            if c == NC - 1:
                q0 = (u // 2) * TQ
                l = o[DH:DH + 1, :]
                br = (2 * k) // H
                gg = g_scr[pl.ds(pl.multiple_of(br * 8, 8), 1), q0:q0 + TQ]
                on = o[0:DH, :] * (gg / l)
                if u % 2 == 0:
                    st["even"] = on
                else:
                    both = jnp.concatenate([st.pop("even"), on], axis=0)
                    oT_scr[pl.ds(pl.multiple_of(k * 2 * DH, 8), 2 * DH), q0:q0 + TQ] = both

        for n in range(max(len(qk_items), len(sm_items))):
            if n < len(qk_items):
                qk(*qk_items[n])
            if n < len(sm_items):
                sm_pv(*sm_items[n])

    run(0, [(0, 0, True)], [])

    def body(k, carry):
        qk_items = [((n + 1) // NC, (n + 1) % NC, n + 1 >= NB) for n in range(NB)]
        sm_items = [(n // NC, n % NC, n < 1) for n in range(NB)]
        run(k, qk_items, sm_items)
        return carry

    lax.fori_loop(0, NSTEP // UNROLL, body, 0)

    woT = woT_scr[...]
    outs = []
    for t, (lo, hi) in enumerate(OTS):
        outT = jnp.dot(woT, oT_scr[:, lo:hi].astype(bf16), preferred_element_type=f32)
        o_v[:, lo:hi] = outT.astype(o_v.dtype)
        cp = pltpu.make_async_copy(o_v.at[:, lo:hi], o_hbm.at[:, lo:hi], sem_out.at[t])
        cp.start()
        outs.append(cp)
    for cp in outs:
        cp.wait()


@jax.jit
def pallas_gated_mix__mha_block__mha_block__prompt_kernel(
    A_x: jax.Array,
    A_wqkv: jax.Array,
    A_wo: jax.Array,
    B_x: jax.Array,
    B_wqkv: jax.Array,
    B_wo: jax.Array,
    gate_w: jax.Array,
):
    del B_x
    bf16 = jnp.bfloat16
    f32 = jnp.float32
    xT = A_x.reshape(S, D).T
    outT = pl.pallas_call(
        _kernel,
        out_shape=jax.ShapeDtypeStruct((D, S), bf16),
        in_specs=[pl.BlockSpec(memory_space=pl.ANY)] * 6,
        out_specs=pl.BlockSpec(memory_space=pl.ANY),
        scratch_shapes=[
            pltpu.VMEM((D, S), bf16),
            pltpu.VMEM((D, 3 * D), bf16),
            pltpu.VMEM((D, 3 * D), bf16),
            pltpu.VMEM((D, D), bf16),
            pltpu.VMEM((D, D), bf16),
            pltpu.VMEM((D,), bf16),
            pltpu.VMEM((D, S), bf16),
            pltpu.SemaphoreType.DMA((6 + len(XCS),)),
            pltpu.SemaphoreType.DMA((len(OTS),)),
            pltpu.VMEM((D, 2 * D), bf16),
            pltpu.VMEM((S, NH * HP), bf16),
            pltpu.VMEM((NH, 128, S), bf16),
            pltpu.VMEM((NH * HP, S), bf16),
            pltpu.VMEM((2 * D, S), f32),
            pltpu.VMEM((16, S), f32),
            pltpu.VMEM((CK, TQ), f32),
        ],
        compiler_params=pltpu.CompilerParams(vmem_limit_bytes=100 * 1024 * 1024),
    )(xT, A_wqkv, B_wqkv, A_wo, B_wo, gate_w)
    return outT.T.reshape(1, S, D)
```

```python
import math

import jax
import jax.numpy as jnp
from jax import lax
from jax.experimental import pallas as pl
from jax.experimental.pallas import tpu as pltpu

S = 2048
D = 448
H = 16
DH = 28
HP = 32
NH = 2 * H
GW = 4 * DH
TQ = 1024
NSTEP = NH * (S // TQ)
CK = 128
NC = S // CK
UNROLL = 4
NB = UNROLL * NC
WQ = 512
XCS = ((0, 512), (512, 1024), (1024, 1536), (1536, 2048))
OTS = ((0, 128), (128, 640), (640, 1152), (1152, 1664), (1664, 1920), (1920, 2048))


def _kernel(x_hbm, wa_hbm, wb_hbm, woa_hbm, wob_hbm, gw_hbm, o_hbm,
            x_v, wa_v, wb_v, woa_v, wob_v, gw_v, o_v, sem_in, sem_out,
            woT_scr, k_scr, q_scr, vT_scr, oT_scr, g_scr, s_carry):
    f32 = jnp.float32
    bf16 = jnp.bfloat16

    pairs = [(wa_hbm.at[:, 0:WQ], wa_v.at[:, 0:WQ])]
    pairs += [(x_hbm.at[:, lo:hi], x_v.at[:, lo:hi]) for lo, hi in XCS]
    pairs += [(wa_hbm.at[:, WQ:3 * D], wa_v.at[:, WQ:3 * D]), (gw_hbm, gw_v), (wb_hbm, wb_v),
              (woa_hbm, woa_v), (wob_hbm, wob_v)]
    copies = [pltpu.make_async_copy(src, dst, sem_in.at[n]) for n, (src, dst) in enumerate(pairs)]
    for cp in copies:
        cp.start()
    c_waq = copies[0]
    c_x = copies[1:1 + len(XCS)]
    c_war, c_gw, c_wb, c_woa, c_wob = copies[1 + len(XCS):]

    qscale = (DH ** -0.5) * math.log2(math.e)

    def store_q(br, qT, lo, hi):
        q16 = (qT * qscale).astype(bf16)
        r = lax.broadcasted_iota(jnp.int32, (GW, hi - lo), 0)
        zpad = jnp.zeros((128 - GW, hi - lo), bf16)
        for g4 in range(4):
            qg = q16[g4 * GW:(g4 + 1) * GW, :]
            for j in range(4):
                qm = jnp.where((r >= j * DH) & (r < (j + 1) * DH), qg, jnp.zeros_like(qg))
                q_scr[br * H + g4 * 4 + j, :, lo:hi] = jnp.concatenate([qm, zpad], axis=0)

    c_waq.wait()
    wqT = wa_v[:, 0:WQ].astype(f32).T[0:D, :].astype(bf16)
    for n, (lo, hi) in enumerate(XCS):
        c_x[n].wait()
        if n == len(XCS) - 1:
            c_war.wait()
            c_gw.wait()
        store_q(0, jnp.dot(wqT, x_v[:, lo:hi], preferred_element_type=f32), lo, hi)
    xT = x_v[...]
    for br, w_v in enumerate((wa_v, wb_v)):
        wt = w_v[...].astype(f32).T.astype(bf16)
        kT = jnp.dot(wt[D:2 * D, :], xT, preferred_element_type=f32)
        kT = jnp.concatenate([kT, jnp.zeros((128 - GW, S), f32)], axis=0)
        for g4 in range(4):
            k_scr[:, (br * 4 + g4) * 128:(br * 4 + g4 + 1) * 128] = (
                kT[g4 * GW:g4 * GW + 128, :].T.astype(bf16))
        if br == 1:
            store_q(1, jnp.dot(wt[0:D, :], xT, preferred_element_type=f32), 0, S)
        wvT = wt[2 * D:3 * D, :]
        if br == 0:
            c_wb.wait()
            c_woa.wait()
            c_wob.wait()
            wvT = jnp.concatenate(
                [wvT, jnp.broadcast_to(gw_v[...].reshape(1, D), (16, D))], axis=0)
        vT = jnp.dot(wvT, xT, preferred_element_type=f32)
        if br == 0:
            g = jax.nn.sigmoid(vT[D:D + 1, :])
            g_scr[0:1, :] = g
            g_scr[8:9, :] = 1.0 - g
        pad = jnp.where(lax.broadcasted_iota(jnp.int32, (HP - DH, S), 0) == 0, 1.0, 0.0)
        for h in range(H):
            dst = (br * H + h) * HP
            vT_scr[dst:dst + HP, :] = jnp.concatenate(
                [vT[h * DH:(h + 1) * DH, :], pad], axis=0).astype(bf16)
        if br == 0:
            woT_scr[:, 0:D] = woa_v[...].astype(f32).T.astype(bf16)
            woT_scr[:, D:2 * D] = wob_v[...].astype(f32).T.astype(bf16)

    def get_q(k, u):
        if u == UNROLL:
            k = jnp.minimum(k + 1, NSTEP // UNROLL - 1)
            u = 0
        q0 = (u // 2) * TQ
        koff = pl.multiple_of(lax.shift_right_logical(k, 1) * 128, 128)
        return q_scr[2 * k + u % 2, :, q0:q0 + TQ], koff

    def run(k, qk_items, sm_items):
        st = {}
        sbuf = {}

        def qk(u, c, to_carry):
            if ("q", u) not in st:
                st[("q", u)] = get_q(k, u)
            qm, koff = st[("q", u)]
            kc = k_scr[c * CK:(c + 1) * CK, pl.ds(koff, 128)]
            s = jnp.dot(kc, qm, preferred_element_type=f32)
            if to_carry:
                s_carry[...] = s
            else:
                sbuf[(u, c)] = s

        def sm_pv(u, c, from_carry):
            h = 2 * k + u % 2
            s = s_carry[...] if from_carry else sbuf.pop((u, c))
            m, o = st.get(("s", u), (None, None))
            mm = jnp.max(s, axis=0, keepdims=True)
            m_new = mm if m is None else jnp.maximum(m, mm)
            p = jnp.exp2(s - m_new).astype(bf16)
            vh = vT_scr[pl.ds(pl.multiple_of(h * HP, HP), HP), c * CK:(c + 1) * CK]
            pv = jnp.dot(vh, p, preferred_element_type=f32)
            o = pv if o is None else o * jnp.exp2(m - m_new) + pv
            st[("s", u)] = (m_new, o)
            if c == NC - 1:
                q0 = (u // 2) * TQ
                oT_scr[pl.ds(pl.multiple_of(h * HP, HP), HP), q0:q0 + TQ] = o

        for n in range(max(len(qk_items), len(sm_items))):
            if n < len(qk_items):
                qk(*qk_items[n])
            if n < len(sm_items):
                sm_pv(*sm_items[n])

    run(jnp.int32(0), [(0, 0, True)], [])

    def body(k, carry):
        qk_items = [((n + 1) // NC, (n + 1) % NC, n + 1 >= NB) for n in range(NB)]
        sm_items = [(n // NC, n % NC, n < 1) for n in range(NB)]
        run(k, qk_items, sm_items)
        return carry

    lax.fori_loop(0, NSTEP // UNROLL, body, 0)

    woT = woT_scr[...]
    outs = []
    for t, (lo, hi) in enumerate(OTS):
        parts = []
        for h in range(NH):
            o = oT_scr[h * HP:(h + 1) * HP, lo:hi]
            gg = g_scr[(h // H) * 8:(h // H) * 8 + 1, lo:hi]
            parts.append(o[0:DH, :] * (gg / o[DH:DH + 1, :]))
        on = jnp.concatenate(parts, axis=0).astype(bf16)
        outT = jnp.dot(woT, on, preferred_element_type=f32)
        o_v[:, lo:hi] = outT.astype(o_v.dtype)
        cp = pltpu.make_async_copy(o_v.at[:, lo:hi], o_hbm.at[:, lo:hi], sem_out.at[t])
        cp.start()
        outs.append(cp)
    for cp in outs:
        cp.wait()


@jax.jit
def pallas_gated_mix__mha_block__mha_block__prompt_kernel(
    A_x: jax.Array,
    A_wqkv: jax.Array,
    A_wo: jax.Array,
    B_x: jax.Array,
    B_wqkv: jax.Array,
    B_wo: jax.Array,
    gate_w: jax.Array,
):
    del B_x
    bf16 = jnp.bfloat16
    f32 = jnp.float32
    xT = A_x.reshape(S, D).T
    outT = pl.pallas_call(
        _kernel,
        out_shape=jax.ShapeDtypeStruct((D, S), bf16),
        in_specs=[pl.BlockSpec(memory_space=pl.ANY)] * 6,
        out_specs=pl.BlockSpec(memory_space=pl.ANY),
        scratch_shapes=[
            pltpu.VMEM((D, S), bf16),
            pltpu.VMEM((D, 3 * D), bf16),
            pltpu.VMEM((D, 3 * D), bf16),
            pltpu.VMEM((D, D), bf16),
            pltpu.VMEM((D, D), bf16),
            pltpu.VMEM((D,), bf16),
            pltpu.VMEM((D, S), bf16),
            pltpu.SemaphoreType.DMA((6 + len(XCS),)),
            pltpu.SemaphoreType.DMA((len(OTS),)),
            pltpu.VMEM((D, 2 * D), bf16),
            pltpu.VMEM((S, NH * HP), bf16),
            pltpu.VMEM((NH, 128, S), bf16),
            pltpu.VMEM((NH * HP, S), bf16),
            pltpu.VMEM((NH * HP, S), f32),
            pltpu.VMEM((16, S), f32),
            pltpu.VMEM((CK, TQ), f32),
        ],
        compiler_params=pltpu.CompilerParams(vmem_limit_bytes=100 * 1024 * 1024),
    )(xT, A_wqkv, B_wqkv, A_wo, B_wo, gate_w)
    return outT.T.reshape(1, S, D)
```
